```python
import jax
import jax.numpy as jnp

def _softmax(x, axis=-1):
    return jax.nn.softmax(x, axis=axis)
def _gelu(x):
    return jax.nn.gelu(x, approximate=True)
def _silu(x):
    return jax.nn.silu(x)
def _sigmoid(x):
    return jax.nn.sigmoid(x)
def _layernorm(x, axis=-1, eps=1e-5):
    m = jnp.mean(x, axis=axis, keepdims=True)
    v = jnp.var(x, axis=axis, keepdims=True)
    return (x - m) / jnp.sqrt(v + eps)
def _scatter_add(tgt, idx, src, axis=0):
    return tgt.at[idx].add(src)
def _segment_sum(src, seg, n):
    return jax.ops.segment_sum(src, seg, n)
class _Rng:
    def __init__(self, key):
        self._k = key
    def _next(self):
        self._k, sub = jax.random.split(self._k)
        return sub
    def normal(self, shape):
        return jax.random.normal(self._next(), shape, dtype=jnp.bfloat16)
    def randint(self, lo, hi, shape):
        return jax.random.randint(self._next(), shape, lo, hi, dtype=jnp.int32)
    def uniform(self, shape, lo=0.0, hi=1.0):
        return jax.random.uniform(self._next(), shape, jnp.bfloat16, lo, hi)
    def permutation(self, n):
        return jax.random.permutation(self._next(), n)


kernel_name = 'standalone__layernorm_linear__prompt'

def setup_inputs():
    _rng = _Rng(jax.random.key(int.from_bytes(__import__("os").urandom(4), "little")))
    _w = (lambda a: (lambda t: t.astype(jnp.bfloat16) if jnp.issubdtype(t.dtype, jnp.floating) else t)(jnp.asarray(a)))
    B, S, D = 2, 2048, 1024
    return {
        "x": _w((lambda *s: _rng.normal(s) * 0.05)(B, S, D)),
        "g": _w((lambda *s: _rng.normal(s) * 0.05)(D) + 1.0),
        "b": _w((lambda *s: _rng.normal(s) * 0.05)(D)),
        "w": _w((lambda *s: _rng.normal(s) * 0.05)(D, D)),
    }

def reference(x, g, b, w):
    return (_layernorm(x, axis=-1) * g + b) @ w
```

```python
import jax
import jax.numpy as jnp
import jax.experimental.pallas as pl
import jax.experimental.pallas.tpu as pltpu

_EPS = 1e-5

_PRO = (320, 352, 352)
_BM = 1024
_NLOOP = 2
_TAIL = (512, 256, 128, 64, 64)
_KGROUPS = (256, 256, 256, 256)
_LN_ROWS = 128


def _layernorm(x_bf16, g, b):
    x = x_bf16.astype(jnp.float32)
    mean = jnp.mean(x, axis=-1, keepdims=True)
    xc = x - mean
    var = jnp.mean(xc * xc, axis=-1, keepdims=True)
    return (xc * jax.lax.rsqrt(var + _EPS) * g + b).astype(jnp.bfloat16)


@jax.jit
def pallas_standalone__layernorm_linear__prompt_kernel(
    x: jax.Array,
    g: jax.Array,
    b: jax.Array,
    w: jax.Array,
):
    B, S, D = x.shape
    M = B * S
    N = w.shape[1]
    chunks = list(_PRO) + [_BM] * (_NLOOP + 1)
    assert sum(chunks) == M and sum(_KGROUPS) == D and sum(_TAIL) == _BM
    starts = [sum(chunks[:i]) for i in range(len(chunks))]
    n, P, nw = len(chunks), len(_PRO), len(_KGROUPS)
    kst = [sum(_KGROUPS[:i]) for i in range(nw)]
    PR = sum(_PRO)
    R0 = chunks[0]

    def kernel(x_hbm, g_hbm, b_hbm, w_hbm, o_hbm, xbuf, lnp, lnl, wbuf, obuf, gbuf, bbuf, acc, sem_in, sem_out):
        def xcopy(i, start, size):
            return pltpu.make_async_copy(x_hbm.at[pl.ds(start, size)], xbuf.at[pl.ds(start, size)],
                                         sem_in.at[2 + nw + i])

        def wcopy(j):
            ks = pl.ds(kst[j], _KGROUPS[j])
            return pltpu.make_async_copy(w_hbm.at[ks, :], wbuf.at[ks, :], sem_in.at[2 + j])

        def ocopy(i, start, size):
            return pltpu.make_async_copy(obuf.at[pl.ds(start, size)], o_hbm.at[pl.ds(start, size)], sem_out.at[i])

        gcopy = pltpu.make_async_copy(g_hbm, gbuf, sem_in.at[0])
        bcopy = pltpu.make_async_copy(b_hbm, bbuf, sem_in.at[1])

        gcopy.start()
        bcopy.start()
        xcopy(0, starts[0], chunks[0]).start()
        for j in range(nw):
            wcopy(j).start()
        for i in range(1, n):
            xcopy(i, starts[i], chunks[i]).start()

        gcopy.wait()
        bcopy.wait()
        xcopy(0, starts[0], chunks[0]).wait()
        gamma = gbuf[...].astype(jnp.float32).reshape(1, D)
        beta = bbuf[...].astype(jnp.float32).reshape(1, D)

        def layernorm(src_start, size, dst, dst_start):
            off = 0
            while off < size:
                c = min(_LN_ROWS, size - off)
                dst[pl.ds(dst_start + off, c), :] = _layernorm(xbuf[pl.ds(src_start + off, c), :], gamma, beta)
                off += c

        def matmul(src, src_start, out_start, size):
            obuf[pl.ds(out_start, size), :] = jnp.dot(
                src[pl.ds(src_start, size), :], wbuf[...], preferred_element_type=jnp.float32
            ).astype(jnp.bfloat16)

        layernorm(0, R0, lnp, 0)
        for j in range(nw):
            last = j == nw - 1
            wcopy(j).wait()
            if last:
                xcopy(1, starts[1], chunks[1]).wait()
            ks = pl.ds(kst[j], _KGROUPS[j])
            p = jnp.dot(lnp[pl.ds(0, R0), ks], wbuf[ks, :], preferred_element_type=jnp.float32)
            if j == 0:
                acc[...] = p
            elif not last:
                acc[...] += p
            else:
                obuf[pl.ds(0, R0), :] = (acc[...] + p).astype(jnp.bfloat16)
                layernorm(starts[1], chunks[1], lnp, starts[1])
                ocopy(0, 0, R0).start()

        for i in range(1, P):
            xcopy(i + 1, starts[i + 1], chunks[i + 1]).wait()
            matmul(lnp, starts[i], starts[i], chunks[i])
            if i + 1 < P:
                layernorm(starts[i + 1], chunks[i + 1], lnp, starts[i + 1])
            else:
                layernorm(starts[i + 1], _BM, lnl.at[0], 0)
            ocopy(i, starts[i], chunks[i]).start()

        def body(t, carry):
            st = pl.multiple_of(PR + t * _BM, _BM)
            nst = pl.multiple_of(PR + (t + 1) * _BM, _BM)
            xcopy(P + t + 1, nst, _BM).wait()
            matmul(lnl.at[t % 2], 0, st, _BM)
            layernorm(nst, _BM, lnl.at[(t + 1) % 2], 0)
            ocopy(P + t, st, _BM).start()
            return carry

        jax.lax.fori_loop(0, _NLOOP, body, None)

        off = 0
        for ti, sz in enumerate(_TAIL):
            matmul(lnl.at[_NLOOP % 2], off, starts[n - 1] + off, sz)
            ocopy(n - 1 + ti, starts[n - 1] + off, sz).start()
            off += sz

        for i in range(n - 1):
            ocopy(i, starts[i], chunks[i]).wait()
        off = 0
        for ti, sz in enumerate(_TAIL):
            ocopy(n - 1 + ti, starts[n - 1] + off, sz).wait()
            off += sz

    out = pl.pallas_call(
        kernel,
        in_specs=[pl.BlockSpec(memory_space=pl.ANY)] * 4,
        out_specs=pl.BlockSpec(memory_space=pl.ANY),
        out_shape=jax.ShapeDtypeStruct((M, N), x.dtype),
        scratch_shapes=[
            pltpu.VMEM((M, D), jnp.bfloat16),
            pltpu.VMEM((PR, D), jnp.bfloat16),
            pltpu.VMEM((2, _BM, D), jnp.bfloat16),
            pltpu.VMEM((D, N), jnp.bfloat16),
            pltpu.VMEM((M, N), jnp.bfloat16),
            pltpu.VMEM((D,), jnp.bfloat16),
            pltpu.VMEM((D,), jnp.bfloat16),
            pltpu.VMEM((R0, N), jnp.float32),
            pltpu.SemaphoreType.DMA((2 + nw + n,)),
            pltpu.SemaphoreType.DMA((n - 1 + len(_TAIL),)),
        ],
        compiler_params=pltpu.CompilerParams(
            vmem_limit_bytes=100 * 2**20,
            flags={"XLA_TPU_EVENLY_DISTRIBUTE_CRITICAL_NODES": True},
            disable_bounds_checks=True,
        ),
    )(x.reshape(M, D), g, b, w)
    return out.reshape(B, S, N)
```
